```python
import os as _os
_os.environ.setdefault("JAX_PLATFORMS", "cpu")
import jax
import jax.numpy as jnp

def _softmax(x, axis=-1):
    return jax.nn.softmax(x, axis=axis)
def _gelu(x):
    return jax.nn.gelu(x, approximate=True)
def _silu(x):
    return jax.nn.silu(x)
def _sigmoid(x):
    return jax.nn.sigmoid(x)
def _layernorm(x, axis=-1, eps=1e-5):
    m = jnp.mean(x, axis=axis, keepdims=True)
    v = jnp.var(x, axis=axis, keepdims=True)
    return (x - m) / jnp.sqrt(v + eps)
def _scatter_add(tgt, idx, src, axis=0):
    return tgt.at[idx].add(src)
def _segment_sum(src, seg, n):
    return jax.ops.segment_sum(src, seg, n)
class _Rng:
    def __init__(self, key):
        self._k = key
    def _next(self):
        self._k, sub = jax.random.split(self._k)
        return sub
    def normal(self, shape):
        return jax.random.normal(self._next(), shape, dtype=jnp.bfloat16)
    def randint(self, lo, hi, shape):
        return jax.random.randint(self._next(), shape, lo, hi, dtype=jnp.int32)
    def uniform(self, shape, lo=0.0, hi=1.0):
        return jax.random.uniform(self._next(), shape, jnp.bfloat16, lo, hi)
    def permutation(self, n):
        return jax.random.permutation(self._next(), n)


kernel_name = 'standalone__detection_seg_fpn_lateral__vision'

def setup_inputs():
    _rng = _Rng(jax.random.key(int.from_bytes(__import__("os").urandom(4), "little")))
    _w = (lambda a: (lambda t: t.astype(jnp.bfloat16) if jnp.issubdtype(t.dtype, jnp.floating) else t)(jnp.asarray(a)))
    H = W = (256 // 2) * 2
    C = 384
    k = 1
    return {
        "c_fine": _w((lambda *s: _rng.normal(s) * 0.05)(1, H, W, C)),
        "p_coarse": _w((lambda *s: _rng.normal(s) * 0.05)(1, H // 2, W // 2, C)),
        "w_lat": _w((lambda *s: _rng.normal(s) * 0.05)(C, C)),
        "w_out": _w((lambda *s: _rng.normal(s) * 0.05)(k, k, C, C)),
    }

def reference(c_fine, p_coarse, w_lat, w_out):
    B, H, W, C = c_fine.shape
    k = 1
    lat = jnp.einsum("bhwc,cd->bhwd", c_fine, w_lat)
    up = jnp.repeat(jnp.repeat(p_coarse, 2, axis=1), 2, axis=2)
    m = lat + up
    pad = k // 2
    mp = jnp.pad(m, ((0, 0), (pad, pad), (pad, pad), (0, 0)))
    o = None
    for di in range(k):
        for dj in range(k):
            t = jnp.einsum("bhwc,cd->bhwd", mp[:, di:di + H, dj:dj + W, :], w_out[di, dj])
            o = t if o is None else o + t
    return o
```

```python
import jax, jax.numpy as jnp
from jax import lax
from jax.experimental import pallas as pl
from jax.experimental.pallas import tpu as pltpu
F32, BF16, U32 = jnp.float32, jnp.bfloat16, jnp.uint32


def divmod2(x, n):
    assert n & (n - 1) == 0
    return x >> (n.bit_length() - 1), x & (n - 1)


def make(NS=8, S=8, PX=64, R=32, rs=2, WR=32, cb=2, c0=1, pb=1, pb_late=8, ring=2, w0=8, wb=2, inplace=False,
         compute=True, rprio=(0, 1), vmem=127, flags=None, nochecks=True, tail=0):
    def fn(c, p, wl, wo):
        B, H, W, C = c.shape
        N = B * H * W
        L = N // NS
        G = NS // S
        KX = W // PX
        T = N // (S * 2 * PX)
        gC = 1 + -(-(T - c0) // cb)
        nG = gC + max(0, -(-(T - tail - gC * pb) // pb_late))
        sw = nG - 1

        def c_end(g):
            return jnp.clip(c0 + (g - 1) * cb, 0, T)

        def p_end(g):
            e = jnp.minimum(jnp.minimum(g, gC) * pb + jnp.maximum(g - gC, 0) * pb_late, T - tail)
            return jnp.where(g > nG, T, e) if tail else e

        def w_end(s):
            return jnp.where(s > sw, jnp.minimum(w0 + (s - 1 - sw) * wb, s - 1), 0)

        def pos(t):
            g, k = divmod2(t, T // G)
            r, x = divmod2(k, KX)
            return g * S, r * (2 * W) + x * PX, k * (PX // 2)

        def kern(c_hbm, p_hbm, wl_hbm, wo_hbm, o_hbm, cbuf, pbuf, obuf, wl_ref, wo_ref, wc_ref, q_ref, rsem, wsem):
            ob = cbuf if inplace else obuf

            def read(src, dst, s0, row, sem):
                for j in range(S // rs):
                    ix = (pl.ds(s0 + j * rs, rs), pl.ds(pl.multiple_of(row, R), R))
                    pltpu.make_async_copy(src.at[ix], dst.at[ix], sem).start(priority=rprio[j % len(rprio)])

            def start_group(g, slot):
                sem = rsem.at[slot]

                def pbody(t, _):
                    s0, _, prow = pos(t)
                    for i in range(PX // 2 // R):
                        read(p_hbm, pbuf, s0, prow + i * R, sem)
                lax.fori_loop(p_end(g), p_end(g + 1), pbody, None)

                def cbody(t, _):
                    s0, row, _ = pos(t)
                    for h in range(2):
                        for i in range(PX // R):
                            read(c_hbm, cbuf, s0, row + h * W + i * R, sem)
                lax.fori_loop(c_end(g), c_end(g + 1), cbody, None)

            def wait_group(g, slot):
                for n, rows in ((p_end(g + 1) - p_end(g), PX // 2), (c_end(g + 1) - c_end(g), 2 * PX)):
                    d = cbuf.at[pl.ds(0, S), pl.ds(0, rows)]
                    lax.fori_loop(0, n, lambda i, _: pltpu.make_async_copy(d, d, rsem.at[slot]).wait(), None)

            def start_writes(lo, hi):
                def body(t, _):
                    s0, row, _ = pos(t)
                    for h in range(2):
                        for i in range(PX // WR):
                            ix = (pl.ds(s0, S), pl.ds(pl.multiple_of(row + h * W + i * WR, WR), WR))
                            pltpu.make_async_copy(ob.at[ix], o_hbm.at[ix], wsem).start()
                lax.fori_loop(lo, hi, body, None)

            wcp = [pltpu.make_async_copy(wl_hbm, wl_ref, wsem), pltpu.make_async_copy(wo_hbm, wo_ref, wsem)]
            wcp[0].start(priority=0)
            wcp[1].start(priority=1)
            lax.fori_loop(0, ring, lambda g, _: start_group(g, g), None)
            wcp[0].wait()
            wcp[1].wait()
            wc_ref[...] = jnp.dot(wl_ref[...], wo_ref[...], preferred_element_type=F32).astype(BF16)

            def step(s, slot):
                @pl.when(s <= nG)
                def _():
                    wait_group(s, slot)
                    start_group(s + ring, slot)
                start_writes(w_end(s), w_end(s + 1))
                nxt = jnp.where(slot == ring - 1, 0, slot + 1)
                if not compute:
                    return nxt
                s0, row, prow = pos(s)
                M = S * PX
                pr = pbuf[pl.ds(s0, S), pl.ds(pl.multiple_of(prow, PX // 2), PX // 2), :].reshape(M // 2, C)
                q = jnp.dot(pr, wo_ref[...], preferred_element_type=F32)
                for j in range(C // 128):
                    q_ref[j, pl.ds(0, M // 2, stride=2), :] = q[:, j * 128:(j + 1) * 128]
                    q_ref[j, pl.ds(1, M // 2, stride=2), :] = q[:, j * 128:(j + 1) * 128]
                ixs = [(pl.ds(s0, S), pl.ds(pl.multiple_of(row + h * W, PX), PX), slice(None)) for h in range(2)]
                xs = [cbuf[ix].reshape(M, C) for ix in ixs]
                for h in range(2):
                    up = jnp.concatenate([q_ref[j] for j in range(C // 128)], axis=1)
                    o = jnp.dot(xs[h], wc_ref[...], preferred_element_type=F32) + up
                    ob[ixs[h]] = o.astype(BF16).reshape(S, PX, C)
                return nxt

            lax.fori_loop(0, T, step, jnp.int32(0))
            start_writes(w_end(T), T)
            pltpu.make_async_copy(ob, o_hbm, wsem).wait()

        any_ = pl.BlockSpec(memory_space=pl.ANY)
        out = pl.pallas_call(
            kern,
            in_specs=[any_] * 4,
            out_specs=any_,
            out_shape=jax.ShapeDtypeStruct((NS, L, C), BF16),
            scratch_shapes=[pltpu.VMEM((NS, L, C), BF16), pltpu.VMEM((NS, L // 4, C), BF16),
                            pltpu.VMEM((1, 16, C) if inplace else (NS, L, C), BF16),
                            pltpu.VMEM((C, C), BF16), pltpu.VMEM((C, C), BF16), pltpu.VMEM((C, C), BF16),
                            pltpu.VMEM((C // 128, S * PX, 128), F32),
                            pltpu.SemaphoreType.DMA((ring,)), pltpu.SemaphoreType.DMA(())],
            compiler_params=pltpu.CompilerParams(vmem_limit_bytes=vmem * 2**20, flags=flags,
                                                 disable_bounds_checks=nochecks),
        )(c.reshape(NS, L, C), p.reshape(NS, L // 4, C), wl, wo.reshape(C, C))
        return out.reshape(B, H, W, C)
    return fn


_fn = make(NS=16, pb_late=16)


@jax.jit
def pallas_standalone__detection_seg_fpn_lateral__vision_kernel(c_fine, p_coarse, w_lat, w_out):
    return _fn(c_fine, p_coarse, w_lat, w_out)
```

```python
import jax
import jax.numpy as jnp
from jax import lax
import jax.experimental.pallas as pl
import jax.experimental.pallas.tpu as pltpu

_BANDS = 16
_S = 8
_PX = 64
_READ_PX = 16
_READ_HI = 2
_WRITE_PX = 32
_AHEAD = 3
_READ_EIGHTHS = 29
_FIRST_WRITES = 20
_WRITES_PER_STEP = 4
_HEAD_UNITS = 16
_TAIL_UNITS = 8
_LANES = 128


def _divmod_pow2(x, n):
    assert n & (n - 1) == 0
    return x >> (n.bit_length() - 1), x & (n - 1)


def _select(pred, a, b):
    if isinstance(pred, bool):
        return a if pred else b
    return jnp.where(pred, a, b)


def _minimum(a, b):
    return _select(a < b, a, b)


@jax.jit
def pallas_standalone__detection_seg_fpn_lateral__vision_kernel(
    c_fine: jax.Array,
    p_coarse: jax.Array,
    w_lat: jax.Array,
    w_out: jax.Array,
):
    B, H, W, C = c_fine.shape
    dtype = c_fine.dtype
    band = B * H * W // _BANDS
    assert band % (2 * W) == 0 and W % _PX == 0 and C % _LANES == 0
    assert w_out.shape == (1, 1, C, C)
    M = _S * _PX
    units = B * H * W // M
    tiles = units // 2
    row_units = 2 * W // _PX

    def locate(u, tile_order):
        g, k = _divmod_pow2(u, band // _PX)
        r, x = _divmod_pow2(k, row_units)
        tiled = r * (2 * W) + (x & 1) * W + (x >> 1) * _PX
        return g * _S, _select(tile_order, tiled, k * _PX), k * (_PX // 4)

    def units_needed(t, tile_order):
        return 2 * t + 2 if tile_order else (2 * t // row_units + 1) * row_units

    def reads_before(g):
        end = _minimum(((g * _READ_EIGHTHS) >> 3) - 1, units - 1)
        return _select(g > 0, end, 0)

    groups = next(g for g in range(tiles) if reads_before(g) == units - 1)
    last_read_step = groups - 1 - _AHEAD
    switch_step = groups - 2

    def writes_through(s):
        done = _select(2 * s >= units - _TAIL_UNITS, 2 * s, 2 * s & -row_units)
        paced = _FIRST_WRITES + _WRITES_PER_STEP * (s - switch_step)
        return _select(s >= switch_step, _minimum(paced, done), 0)

    assert _HEAD_UNITS % row_units == 0 and _TAIL_UNITS % row_units == 0
    assert 0 <= last_read_step and switch_step < tiles - 1
    for t in range(switch_step):
        assert reads_before(t + 1) >= units_needed(t, 2 * t < _HEAD_UNITS)

    def box(band0, bands, px0, px):
        if not isinstance(px0, int):
            px0 = pl.multiple_of(px0, _READ_PX)
        return pl.ds(band0, bands), pl.ds(px0, px)

    def copy(src, dst, index, sem):
        return pltpu.make_async_copy(src.at[index], dst.at[index], sem)

    def for_units(lo, hi, fn):
        lax.fori_loop(lo, hi, lambda u, _: fn(u), None)

    def kernel_function(
        c_hbm, p_hbm, wl_hbm, wo_hbm, o_hbm,
        c_buf, p_buf, o_buf, wl_buf, wo_buf, wc_buf, up_buf, read_sems, sem,
    ):
        def group_sem(g):
            return read_sems.at[g & _AHEAD]

        def start_read(u, g):
            b, px, cpx = locate(u, u < _HEAD_UNITS)
            for src, dst, px0, n in (
                (p_hbm, p_buf, cpx, _PX // 4),
                (c_hbm, c_buf, px, _PX),
            ):
                for i in range(0, n, _READ_PX):
                    hi = box(b, _READ_HI, px0 + i, _READ_PX)
                    lo = box(b + _READ_HI, _S - _READ_HI, px0 + i, _READ_PX)
                    copy(src, dst, hi, group_sem(g)).start(priority=0)
                    copy(src, dst, lo, group_sem(g)).start(priority=1)

        def wait_read(u, g):
            b, px, cpx = locate(u, u < _HEAD_UNITS)
            copy(p_hbm, p_buf, box(b, _S, cpx, _PX // 4), group_sem(g)).wait()
            copy(c_hbm, c_buf, box(b, _S, px, _PX), group_sem(g)).wait()

        def for_group(g, fn):
            for_units(reads_before(g), reads_before(g + 1), lambda u: fn(u, g))

        def start_write(u):
            b, px, _ = locate(u, u >= units - _TAIL_UNITS)
            for i in range(0, _PX, _WRITE_PX):
                copy(o_buf, o_hbm, box(b, _S, px + i, _WRITE_PX), sem).start()

        weights = (
            pltpu.make_async_copy(wl_hbm, wl_buf, sem),
            pltpu.make_async_copy(wo_hbm, wo_buf, sem),
        )
        for w in weights:
            w.start(priority=1)
        lax.fori_loop(0, _AHEAD, lambda g, _: for_group(g, start_read), None)
        for w in weights:
            w.wait()
        wc_buf[...] = jnp.dot(
            wl_buf[...], wo_buf[...], preferred_element_type=jnp.float32
        ).astype(dtype)

        def step(s, _):
            @pl.when(s <= switch_step)
            def _():
                for_group(s, wait_read)
                for_group(s + _AHEAD, start_read)

                @pl.when(s == last_read_step)
                def _():
                    start_read(units - 1, groups)

                @pl.when(s == switch_step)
                def _():
                    for_group(groups - 1, wait_read)

            for_units(writes_through(s - 1), writes_through(s), start_write)

            @pl.when(s == tiles - 1)
            def _():
                wait_read(units - 1, groups)

            b, px, cpx = locate(2 * s, True)
            top = jnp.dot(
                p_buf[box(b, _S, cpx, _PX // 2)].reshape(M // 2, C),
                wo_buf[...],
                preferred_element_type=jnp.float32,
            )
            for j in range(C // _LANES):
                cols = top[:, j * _LANES:(j + 1) * _LANES]
                for parity in range(2):
                    up_buf[j, pl.ds(parity, M // 2, stride=2), :] = cols
            for h in range(2):
                index = box(b, _S, px + h * W, _PX)
                up = jnp.concatenate(
                    [up_buf[j, :M, :] for j in range(C // _LANES)], axis=1
                )
                lat = jnp.dot(
                    c_buf[index].reshape(M, C),
                    wc_buf[...],
                    preferred_element_type=jnp.float32,
                )
                o_buf[index] = (lat + up).astype(dtype).reshape(_S, _PX, C)

        lax.fori_loop(0, tiles, step, None)
        for_units(writes_through(tiles - 1), units, start_write)
        pltpu.make_async_copy(o_buf, o_hbm, sem).wait()

    hbm = pl.BlockSpec(memory_space=pl.ANY)
    out = pl.pallas_call(
        kernel_function,
        in_specs=[hbm] * 4,
        out_specs=hbm,
        out_shape=jax.ShapeDtypeStruct((_BANDS, band, C), dtype),
        scratch_shapes=[
            pltpu.VMEM((_BANDS, band, C), dtype),
            pltpu.VMEM((_BANDS, band // 4, C), dtype),
            pltpu.VMEM((_BANDS, band, C), dtype),
            pltpu.VMEM((C, C), dtype),
            pltpu.VMEM((C, C), dtype),
            pltpu.VMEM((C, C), dtype),
            pltpu.VMEM((C // _LANES, M + 8, _LANES), jnp.float32),
            pltpu.SemaphoreType.DMA((_AHEAD + 1,)),
            pltpu.SemaphoreType.DMA(()),
        ],
        compiler_params=pltpu.CompilerParams(
            vmem_limit_bytes=120 * 1024 * 1024,
            disable_bounds_checks=True,
        ),
    )(
        c_fine.reshape(_BANDS, band, C),
        p_coarse.reshape(_BANDS, band // 4, C),
        w_lat,
        w_out.reshape(C, C),
    )
    return out.reshape(B, H, W, C)
```

```python
import jax
import jax.numpy as jnp
from jax import lax
import jax.experimental.pallas as pl
import jax.experimental.pallas.tpu as pltpu

_BANDS = 16
_S = 8
_PX = 64
_READ_PX = 16
_READ_HI = 2
_WRITE_PX = 32
_AHEAD = 3
_READ_EIGHTHS = 29
_FIRST_WRITES = 20
_WRITES_PER_STEP = 4
_HEAD_UNITS = 16
_TAIL_UNITS = 8
_LANES = 128


def _divmod_pow2(x, n):
    assert n & (n - 1) == 0
    return x >> (n.bit_length() - 1), x & (n - 1)


def _select(pred, a, b):
    if isinstance(pred, bool):
        return a if pred else b
    return jnp.where(pred, a, b)


def _minimum(a, b):
    if isinstance(a, int) and isinstance(b, int):
        return min(a, b)
    return jnp.minimum(a, b)


@jax.jit
def pallas_standalone__detection_seg_fpn_lateral__vision_kernel(
    c_fine: jax.Array,
    p_coarse: jax.Array,
    w_lat: jax.Array,
    w_out: jax.Array,
):
    B, H, W, C = c_fine.shape
    dtype = c_fine.dtype
    band = B * H * W // _BANDS
    assert band % (2 * W) == 0 and W % _PX == 0 and C % _LANES == 0
    assert w_out.shape == (1, 1, C, C)
    M = _S * _PX
    units = B * H * W // M
    tiles = units // 2
    row_units = 2 * W // _PX

    def locate(u, tile_order):
        g, k = _divmod_pow2(u, band // _PX)
        r, x = _divmod_pow2(k, row_units)
        tiled = r * (2 * W) + (x & 1) * W + (x >> 1) * _PX
        return g * _S, _select(tile_order, tiled, k * _PX), k * (_PX // 4)

    def units_needed(t, tile_order):
        return 2 * t + 2 if tile_order else (2 * t // row_units + 1) * row_units

    def reads_before(g):
        end = _minimum(((g * _READ_EIGHTHS) >> 3) - 1, units - 1)
        return _select(g > 0, end, 0)

    groups = next(g for g in range(tiles) if reads_before(g) == units - 1)
    last_read_step = groups - 1 - _AHEAD
    switch_step = groups - 2

    def writes_through(s):
        done = _select(2 * s >= units - _TAIL_UNITS, 2 * s, 2 * s & -row_units)
        paced = _FIRST_WRITES + _WRITES_PER_STEP * (s - switch_step)
        return _minimum(paced, done)

    assert _HEAD_UNITS % row_units == 0 and _TAIL_UNITS % row_units == 0
    assert 0 <= last_read_step and switch_step < tiles - 1
    for t in range(switch_step):
        assert reads_before(t + 1) >= units_needed(t, 2 * t < _HEAD_UNITS)

    def box(band0, bands, px0, px):
        if not isinstance(px0, int):
            px0 = pl.multiple_of(px0, _READ_PX)
        return pl.ds(band0, bands), pl.ds(px0, px)

    def copy(src, dst, index, sem):
        return pltpu.make_async_copy(src.at[index], dst.at[index], sem)

    def for_units(lo, hi, fn):
        lax.fori_loop(lo, hi, lambda u, _: fn(u), None)

    def kernel_function(
        c_hbm, p_hbm, wl_hbm, wo_hbm, o_hbm,
        c_buf, p_buf, o_buf, wl_buf, wo_buf, wc_buf, up_buf, read_sems, sem,
    ):
        def group_sem(g):
            return read_sems.at[g & _AHEAD]

        def start_read(u, g):
            b, px, cpx = locate(u, u < _HEAD_UNITS)
            for src, dst, px0, n in (
                (p_hbm, p_buf, cpx, _PX // 4),
                (c_hbm, c_buf, px, _PX),
            ):
                for i in range(0, n, _READ_PX):
                    hi = box(b, _READ_HI, px0 + i, _READ_PX)
                    lo = box(b + _READ_HI, _S - _READ_HI, px0 + i, _READ_PX)
                    copy(src, dst, hi, group_sem(g)).start(priority=0)
                    copy(src, dst, lo, group_sem(g)).start(priority=1)

        def wait_read(u, g):
            b, px, cpx = locate(u, u < _HEAD_UNITS)
            copy(p_hbm, p_buf, box(b, _S, cpx, _PX // 4), group_sem(g)).wait()
            copy(c_hbm, c_buf, box(b, _S, px, _PX), group_sem(g)).wait()

        def for_group(g, fn):
            for_units(reads_before(g), reads_before(g + 1), lambda u: fn(u, g))

        def start_write(u):
            b, px, _ = locate(u, u >= units - _TAIL_UNITS)
            for i in range(0, _PX, _WRITE_PX):
                copy(o_buf, o_hbm, box(b, _S, px + i, _WRITE_PX), sem).start()

        weights = (
            pltpu.make_async_copy(wl_hbm, wl_buf, sem),
            pltpu.make_async_copy(wo_hbm, wo_buf, sem),
        )
        for w in weights:
            w.start(priority=1)
        lax.fori_loop(0, _AHEAD, lambda g, _: for_group(g, start_read), None)
        for w in weights:
            w.wait()
        wc_buf[...] = jnp.dot(
            wl_buf[...], wo_buf[...], preferred_element_type=jnp.float32
        ).astype(dtype)

        def step(s, _):
            @pl.when(s < switch_step)
            def _():
                for_group(s, wait_read)
                for_group(s + _AHEAD, start_read)

                @pl.when(s == last_read_step)
                def _():
                    start_read(units - 1, groups)

            @pl.when(s == switch_step)
            def _():
                for g in range(switch_step, groups):
                    for u in range(reads_before(g), reads_before(g + 1)):
                        wait_read(u, g)
                start_write(0)
                for_units(1, writes_through(switch_step), start_write)

            @pl.when(s > switch_step)
            def _():
                for_units(writes_through(s - 1), writes_through(s), start_write)

                @pl.when(s == tiles - 1)
                def _():
                    wait_read(units - 1, groups)

            b, px, cpx = locate(2 * s, True)
            top = jnp.dot(
                p_buf[box(b, _S, cpx, _PX // 2)].reshape(M // 2, C),
                wo_buf[...],
                preferred_element_type=jnp.float32,
            )
            for j in range(C // _LANES):
                cols = top[:, j * _LANES:(j + 1) * _LANES]
                for parity in range(2):
                    up_buf[j, pl.ds(parity, M // 2, stride=2), :] = cols
            for h in range(2):
                index = box(b, _S, px + h * W, _PX)
                up = jnp.concatenate(
                    [up_buf[j, :M, :] for j in range(C // _LANES)], axis=1
                )
                lat = jnp.dot(
                    c_buf[index].reshape(M, C),
                    wc_buf[...],
                    preferred_element_type=jnp.float32,
                )
                o_buf[index] = (lat + up).astype(dtype).reshape(_S, _PX, C)

        lax.fori_loop(0, tiles, step, None)
        for_units(writes_through(tiles - 1), units, start_write)
        pltpu.make_async_copy(o_buf, o_hbm, sem).wait()

    hbm = pl.BlockSpec(memory_space=pl.ANY)
    out = pl.pallas_call(
        kernel_function,
        in_specs=[hbm] * 4,
        out_specs=hbm,
        out_shape=jax.ShapeDtypeStruct((_BANDS, band, C), dtype),
        scratch_shapes=[
            pltpu.VMEM((_BANDS, band, C), dtype),
            pltpu.VMEM((_BANDS, band // 4, C), dtype),
            pltpu.VMEM((_BANDS, band, C), dtype),
            pltpu.VMEM((C, C), dtype),
            pltpu.VMEM((C, C), dtype),
            pltpu.VMEM((C, C), dtype),
            pltpu.VMEM((C // _LANES, M + 8, _LANES), jnp.float32),
            pltpu.SemaphoreType.DMA((_AHEAD + 1,)),
            pltpu.SemaphoreType.DMA(()),
        ],
        compiler_params=pltpu.CompilerParams(
            vmem_limit_bytes=120 * 1024 * 1024,
            disable_bounds_checks=True,
        ),
    )(
        c_fine.reshape(_BANDS, band, C),
        p_coarse.reshape(_BANDS, band // 4, C),
        w_lat,
        w_out.reshape(C, C),
    )
    return out.reshape(B, H, W, C)
```
